```python
import os as _os
_os.environ.setdefault('JAX_PLATFORMS', 'cpu')
import jax
import jax.numpy as jnp

def _softmax(x, axis=-1):
    return jax.nn.softmax(x, axis=axis)

def _gelu(x):
    return jax.nn.gelu(x, approximate=True)

def _silu(x):
    return jax.nn.silu(x)

def _sigmoid(x):
    return jax.nn.sigmoid(x)

def _layernorm(x, axis=-1, eps=1e-05):
    m = jnp.mean(x, axis=axis, keepdims=True)
    v = jnp.var(x, axis=axis, keepdims=True)
    return (x - m) / jnp.sqrt(v + eps)

def _scatter_add(tgt, idx, src, axis=0):
    return tgt.at[idx].add(src)

def _segment_sum(src, seg, n):
    return jax.ops.segment_sum(src, seg, n)

class _Rng:

    def __init__(self, key):
        self._k = key

    def _next(self):
        self._k, sub = jax.random.split(self._k)
        return sub

    def normal(self, shape):
        return jax.random.normal(self._next(), shape, dtype=jnp.bfloat16)

    def randint(self, lo, hi, shape):
        return jax.random.randint(self._next(), shape, lo, hi, dtype=jnp.int32)

    def uniform(self, shape, lo=0.0, hi=1.0):
        return jax.random.uniform(self._next(), shape, jnp.bfloat16, lo, hi)

    def permutation(self, n):
        return jax.random.permutation(self._next(), n)
kernel_name = 'adaLN_cond__linear_kernel_hedgehog__geglu_ffn__prompt'

def setup_inputs():
    _rng = _Rng(jax.random.key(int.from_bytes(__import__("os").urandom(4), "little")))
    _w = lambda a: (lambda t: t.astype(jnp.bfloat16) if jnp.issubdtype(t.dtype, jnp.floating) else t)(jnp.asarray(a))

    def _A_setup():
        B, S, D, H = (1, 2048, 512, 32)
        Dh = D // H
        return {'x': _w((lambda *s: _rng.normal(s) * 0.05)(B, S, D)), 'wqkv': _w((lambda *s: _rng.normal(s) * 0.4)(D, 3 * D)), 'w_phi': _w((lambda *s: _rng.normal(s) * 0.4)(H, Dh, Dh) * Dh ** (-0.5)), 'wo': _w((lambda *s: _rng.normal(s) * 0.05)(D, D))}
    _A_in = _A_setup()

    def _B_setup():
        B, S, D, F = (1, 2048, 512, 1792)
        return {'x': _w((lambda *s: _rng.normal(s) * 0.05)(B, S, D)), 'w_gate': _w((lambda *s: _rng.normal(s) * 0.05)(D, F)), 'w_up': _w((lambda *s: _rng.normal(s) * 0.05)(D, F)), 'w_down': _w((lambda *s: _rng.normal(s) * 0.05)(F, D))}
    _B_in = _B_setup()
    return {'A_x': _A_in['x'], 'A_wqkv': _A_in['wqkv'], 'A_w_phi': _A_in['w_phi'], 'A_wo': _A_in['wo'], 'B_x': _B_in['x'], 'B_w_gate': _B_in['w_gate'], 'B_w_up': _B_in['w_up'], 'B_w_down': _B_in['w_down'], 'c': _w((lambda *s: _rng.normal(s) * 0.05)(1, 512) * 8.0), 'w_mod': _w((lambda *s: _rng.normal(s) * 0.05)(512, 6 * 512) * 512 ** (-0.5) * 8.0)}

def reference(A_x, A_wqkv, A_w_phi, A_wo, B_x, B_w_gate, B_w_up, B_w_down, c, w_mod):

    def _A_ref(x, wqkv, w_phi, wo):
        B, S, D = x.shape
        H = 32
        Dh = D // H
        qkv = (lambda x, *d: x.transpose(*d))((x @ wqkv).reshape(B, S, 3, H, Dh), 2, 0, 3, 1, 4)
        q, k, v = (qkv[0], qkv[1], qkv[2])
        pq = jnp.einsum('bhsd,hdf->bhsf', q, w_phi)
        pk = jnp.einsum('bhsd,hdf->bhsf', k, w_phi)
        phi_q = jnp.concatenate([_softmax(pq, axis=-1), _softmax(-pq, axis=-1)], axis=-1)
        phi_k = jnp.concatenate([_softmax(pk, axis=-1), _softmax(-pk, axis=-1)], axis=-1)
        kv = jnp.einsum('bhsf,bhsd->bhfd', phi_k, v)
        z = jnp.einsum('bhsf->bhf', phi_k)
        num = jnp.einsum('bhqf,bhfd->bhqd', phi_q, kv)
        den = jnp.einsum('bhqf,bhf->bhq', phi_q, z)[..., None] + 1e-06
        o = num / den
        return (lambda x, *d: x.transpose(*d))(o, 0, 2, 1, 3).reshape(B, S, D) @ wo

    def _B_ref(x, w_gate, w_up, w_down):
        return _gelu(x @ w_gate) * (x @ w_up) @ w_down
    x = A_x
    mod = (_silu(c) @ w_mod).reshape(c.shape[0], 6, 1, -1)
    sa, ca, ga, sb, cb, gb = (mod[:, 0].copy(), mod[:, 1].copy(), mod[:, 2].copy(), mod[:, 3].copy(), mod[:, 4].copy(), mod[:, 5].copy())
    h = _layernorm(x, axis=-1) * (1 + ca) + sa
    x = x + ga * _A_ref(h, A_wqkv, A_w_phi, A_wo)
    h = _layernorm(x, axis=-1) * (1 + cb) + sb
    x = x + gb * _B_ref(h, B_w_gate, B_w_up, B_w_down)
    return x
```

```python
import functools
import jax
import jax.numpy as jnp
from jax import lax
import jax.experimental.pallas as pl
import jax.experimental.pallas.tpu as pltpu

S = 2048
D = 512
H = 32
DH = 16
F = 1792
NG = 4
NJ = 8
TM = 256
NB = S // TM
FC = 256
NFC = F // FC
EPS = 1e-5

bf16 = jnp.bfloat16
f32 = jnp.float32

_NT = (((1,), (1,)), ((), ()))


def _dot(a, b):
    return jnp.dot(a, b, preferred_element_type=f32)


def _dot_nt(a, b):
    return lax.dot_general(a, b, _NT, preferred_element_type=f32)


def _layernorm_mod(x, scale1p, shift):
    m = jnp.mean(x, axis=-1, keepdims=True)
    xc = x - m
    v = jnp.mean(xc * xc, axis=-1, keepdims=True)
    return xc * lax.rsqrt(v + EPS) * scale1p + shift


def _fold(x):
    return pltpu.roll(x, 4, 0)


def _feature_map_j(pT):
    n = pT.shape[-1]
    t = pT.reshape(8, 8, n)
    mx = jnp.max(t, axis=0)
    mx = jnp.maximum(mx, _fold(mx))
    mn = jnp.min(t, axis=0)
    mn = jnp.minimum(mn, _fold(mn))
    ep = jnp.exp(t - mx[None])
    en = jnp.exp(mn[None] - t)
    sp = jnp.sum(ep, axis=0)
    sp = sp + _fold(sp)
    sn = jnp.sum(en, axis=0)
    sn = sn + _fold(sn)
    return jnp.concatenate([(ep * (1.0 / sp)[None]).reshape(64, n), (en * (1.0 / sn)[None]).reshape(64, n)], axis=0)


def _kernel(x_hbm, wqkv_hbm, wphi_hbm, wo_hbm, wg_hbm, wu_hbm, wd_hbm, c_hbm, wmod_hbm,
            out_hbm,
            x_v, h_v, out_v, wqkv_v, wphi_v, wo_v, wg_v, wu_v, wd_v, c_v, wmod_v,
            wqT_v, wkT_v, wvT_v, kv_acc, z_acc, kvT_v, zb_v, mod_v, x1_v, h2_v,
            sem_x, sem_o, sem_w):
    cp_phi = pltpu.make_async_copy(wphi_hbm, wphi_v, sem_w.at[0])
    cp_wk = pltpu.make_async_copy(wqkv_hbm.at[:, pl.ds(D, D)], wqkv_v.at[:, pl.ds(D, D)], sem_w.at[1])
    cp_c = pltpu.make_async_copy(c_hbm, c_v, sem_w.at[2])
    cp_m0 = pltpu.make_async_copy(wmod_hbm.at[:, pl.ds(0, 2 * D)], wmod_v.at[:, pl.ds(0, 2 * D)], sem_w.at[3])
    cp_wv = pltpu.make_async_copy(wqkv_hbm.at[:, pl.ds(2 * D, D)], wqkv_v.at[:, pl.ds(2 * D, D)], sem_w.at[4])
    cp_wq = pltpu.make_async_copy(wqkv_hbm.at[:, pl.ds(0, D)], wqkv_v.at[:, pl.ds(0, D)], sem_w.at[5])
    cp_m1 = pltpu.make_async_copy(wmod_hbm.at[:, pl.ds(2 * D, 4 * D)], wmod_v.at[:, pl.ds(2 * D, 4 * D)], sem_w.at[6])
    cp_wo = pltpu.make_async_copy(wo_hbm, wo_v, sem_w.at[7])
    cp_wg = pltpu.make_async_copy(wg_hbm, wg_v, sem_w.at[8])
    cp_wu = pltpu.make_async_copy(wu_hbm, wu_v, sem_w.at[9])
    cp_wd = pltpu.make_async_copy(wd_hbm, wd_v, sem_w.at[10])

    def x_copy(i):
        return pltpu.make_async_copy(x_hbm.at[pl.ds(i * TM, TM)], x_v.at[pl.ds(i * TM, TM)], sem_x.at[i])

    def o_copy(i):
        return pltpu.make_async_copy(out_v.at[pl.ds(i * TM, TM)], out_hbm.at[pl.ds(i * TM, TM)], sem_o.at[i])

    cp_phi.start()
    cp_wk.start()
    cp_wv.start()
    cp_c.start()
    cp_m0.start()
    x_copy(0).start()

    cp_phi.wait()
    B = wphi_v[...].reshape(DH * DH, H)
    r1 = lax.broadcasted_iota(jnp.int32, (D, H), 0)
    c1 = lax.broadcasted_iota(jnp.int32, (D, H), 1)
    E1 = jnp.where((r1 // 64) * 4 + (r1 % 4) == c1, 1.0, 0.0).astype(bf16)
    M1 = _dot_nt(E1, B)
    r2 = lax.broadcasted_iota(jnp.int32, (D, DH * DH), 0)
    c2 = lax.broadcasted_iota(jnp.int32, (D, DH * DH), 1)
    M1 = jnp.where(((r2 % 64) // 4) == (c2 % DH), M1, 0.0).astype(bf16)
    r3 = lax.broadcasted_iota(jnp.int32, (DH * DH, 128), 0)
    c3 = lax.broadcasted_iota(jnp.int32, (DH * DH, 128), 1)
    E2 = jnp.where((r3 // DH) == (c3 % DH), 1.0, 0.0).astype(bf16)
    PT = _dot(M1, E2)
    r4 = lax.broadcasted_iota(jnp.int32, (D, 128), 0)
    c4 = lax.broadcasted_iota(jnp.int32, (D, 128), 1)
    PT = jnp.where(((r4 % 128) // 64) * 4 + (r4 % 4) == (c4 // DH), PT, 0.0).astype(bf16)
    pts = [PT[g * 128:(g + 1) * 128] for g in range(NG)]

    cp_wk.wait()
    for g in range(NG):
        wkT_v[g * 128:(g + 1) * 128, :] = _dot_nt(
            pts[g], wqkv_v[:, D + g * 128:D + (g + 1) * 128]).astype(bf16)
    cp_wv.wait()
    for i in range(1, NB):
        x_copy(i).start()
    cp_wq.start()
    wvT_v[...] = wqkv_v[:, 2 * D:3 * D].astype(f32).T.astype(bf16)

    cp_c.wait()
    cp_m0.wait()
    cp_m1.start()
    cp_wo.start()
    cp_wg.start()
    cp_wu.start()
    cp_wd.start()
    cf = c_v[...].astype(f32)
    sc = (cf * jax.nn.sigmoid(cf)).astype(bf16)
    sc8 = jnp.broadcast_to(sc, (8, D))
    mod_v[:, 0:2 * D] = _dot(sc8, wmod_v[:, 0:2 * D])

    kv_acc[...] = jnp.zeros_like(kv_acc)
    z_acc[...] = jnp.zeros_like(z_acc)

    HT = TM // 2

    def ln1_part(i, p):
        r0 = pl.multiple_of(i * TM + p * HT, HT)
        x = x_v[pl.ds(r0, HT), :].astype(f32)
        sa = mod_v[0:1, 0:D]
        ca = mod_v[0:1, D:2 * D]
        h_v[pl.ds(r0, HT), :] = _layernorm_mod(x, 1.0 + ca, sa).astype(bf16)

    def kv_block(i, nxt):
        r0 = pl.multiple_of(i * TM, TM)
        h = h_v[pl.ds(r0, TM), :]
        kT = _dot_nt(wkT_v[...], h)
        if nxt:
            ln1_part(i + 1, 0)
        vT = _dot_nt(wvT_v[...], h).astype(bf16)
        if nxt:
            ln1_part(i + 1, 1)
        for j in range(NJ):
            ph = _feature_map_j(kT[j * 64:(j + 1) * 64])
            zs = ph[:, 0:128]
            for jj in range(1, TM // 128):
                zs = zs + ph[:, jj * 128:(jj + 1) * 128]
            z_acc[j] += zs
            kv_acc[j] += _dot_nt(vT[j * 64:(j + 1) * 64], ph.astype(bf16))

    x_copy(0).wait()
    ln1_part(0, 0)
    ln1_part(0, 1)

    def phase1(i, carry):
        x_copy(i + 1).wait()
        kv_block(i, True)
        return carry

    lax.fori_loop(0, NB - 1, phase1, 0)
    kv_block(NB - 1, False)

    rk = lax.broadcasted_iota(jnp.int32, (64, 128), 0)
    ck = lax.broadcasted_iota(jnp.int32, (64, 128), 1)
    kv_mask = (rk // DH) == (ck % 4)
    for j in range(NJ):
        kvT_v[j] = jnp.where(kv_mask, kv_acc[j], 0.0).astype(bf16)
        z = jnp.sum(z_acc[j], axis=-1, keepdims=True)
        zb_v[j] = jnp.broadcast_to(z, (128, TM))

    cp_wq.wait()
    for g in range(NG):
        wqT_v[g * 128:(g + 1) * 128, :] = _dot_nt(
            pts[g], wqkv_v[:, g * 128:(g + 1) * 128]).astype(bf16)
    cp_m1.wait()
    mod_v[:, 2 * D:6 * D] = _dot(sc8, wmod_v[:, 2 * D:6 * D])
    cp_wo.wait()

    def attn_stages(i):
        r0 = pl.multiple_of(i * TM, TM)
        h = h_v[pl.ds(r0, TM), :]
        qT = _dot_nt(wqT_v[...], h)
        yield
        oTs = []
        for j in range(NJ):
            ph = _feature_map_j(qT[j * 64:(j + 1) * 64])
            den = jnp.sum((ph * zb_v[j]).reshape(16, 8, TM), axis=0)
            den = den + _fold(den)
            rden = 1.0 / (den + 1e-6)
            num = _dot(kvT_v[j], ph.astype(bf16))
            num = num.reshape(4, DH, TM) * rden[0:4, None, :]
            oTs.append(num.reshape(64, TM))
            if j % 4 == 3:
                yield
        oT = jnp.concatenate(oTs, axis=0)
        o = oT.T.astype(bf16)
        yield
        attn = _dot(o, wo_v[...])
        yield
        ga = mod_v[0:1, 2 * D:3 * D]
        sb = mod_v[0:1, 3 * D:4 * D]
        cb = mod_v[0:1, 4 * D:5 * D]
        for p in range(2):
            rp = pl.multiple_of(i * TM + p * HT, HT)
            x = x_v[pl.ds(rp, HT), :].astype(f32)
            x1 = x + ga * attn[p * HT:(p + 1) * HT]
            x1_v[pl.ds(rp, HT), :] = x1
            h2_v[pl.ds(rp, HT), :] = _layernorm_mod(x1, 1.0 + cb, sb).astype(bf16)
            yield

    def ffn_stages(i):
        r0 = pl.multiple_of(i * TM, TM)
        h2 = h2_v[pl.ds(r0, TM), :]
        gb = mod_v[0:1, 5 * D:6 * D]
        acc = None
        for j in range(NFC):
            gt = _dot(h2, wg_v[:, j * FC:(j + 1) * FC])
            up = _dot(h2, wu_v[:, j * FC:(j + 1) * FC])
            a = (jax.nn.gelu(gt, approximate=True) * up).astype(bf16)
            d = _dot(a, wd_v[j * FC:(j + 1) * FC, :])
            acc = d if acc is None else acc + d
            if j < NFC - 1:
                yield
        out_v[pl.ds(r0, TM), :] = (x1_v[pl.ds(r0, TM), :] + gb * acc).astype(bf16)
        o_copy(i).start()
        yield

    for _ in attn_stages(0):
        pass
    cp_wg.wait()
    cp_wu.wait()
    cp_wd.wait()

    def phase2(i, carry):
        fs = ffn_stages(i)
        as_ = attn_stages(i + 1)
        done_a = done_f = False
        while not (done_a and done_f):
            if not done_a:
                try:
                    next(as_)
                except StopIteration:
                    done_a = True
            if not done_f:
                try:
                    next(fs)
                except StopIteration:
                    done_f = True
        return carry

    lax.fori_loop(0, NB - 1, phase2, 0)
    for _ in ffn_stages(NB - 1):
        pass

    for i in range(NB):
        o_copy(i).wait()


@jax.jit
def pallas_adaLN_cond__linear_kernel_hedgehog__geglu_ffn__prompt_kernel(
    A_x, A_wqkv, A_w_phi, A_wo, B_x, B_w_gate, B_w_up, B_w_down, c, w_mod,
):
    x2 = A_x.reshape(S, D)
    wphiT = jnp.transpose(A_w_phi, (1, 2, 0))
    any_spec = pl.BlockSpec(memory_space=pl.ANY)
    out = pl.pallas_call(
        _kernel,
        out_shape=jax.ShapeDtypeStruct((S, D), bf16),
        in_specs=[any_spec] * 9,
        out_specs=any_spec,
        scratch_shapes=[
            pltpu.VMEM((S, D), bf16),
            pltpu.VMEM((S, D), bf16),
            pltpu.VMEM((S, D), bf16),
            pltpu.VMEM((D, 3 * D), bf16),
            pltpu.VMEM((DH, DH, H), bf16),
            pltpu.VMEM((D, D), bf16),
            pltpu.VMEM((D, F), bf16),
            pltpu.VMEM((D, F), bf16),
            pltpu.VMEM((F, D), bf16),
            pltpu.VMEM((1, D), bf16),
            pltpu.VMEM((D, 6 * D), bf16),
            pltpu.VMEM((D, D), bf16),
            pltpu.VMEM((D, D), bf16),
            pltpu.VMEM((D, D), bf16),
            pltpu.VMEM((NJ, 64, 128), f32),
            pltpu.VMEM((NJ, 128, 128), f32),
            pltpu.VMEM((NJ, 64, 128), bf16),
            pltpu.VMEM((NJ, 128, TM), f32),
            pltpu.VMEM((8, 6 * D), f32),
            pltpu.VMEM((S, D), f32),
            pltpu.VMEM((S, D), bf16),
            pltpu.SemaphoreType.DMA((NB,)),
            pltpu.SemaphoreType.DMA((NB,)),
            pltpu.SemaphoreType.DMA((11,)),
        ],
        compiler_params=pltpu.CompilerParams(vmem_limit_bytes=100 * 1024 * 1024),
    )(x2, A_wqkv, wphiT, A_wo, B_w_gate, B_w_up, B_w_down, c, w_mod)
    return out.reshape(1, S, D)
```

```python
import jax
import jax.numpy as jnp
from jax import lax
import jax.experimental.pallas as pl
import jax.experimental.pallas.tpu as pltpu

S = 2048
D = 512
H = 32
DH = 16
F = 1792
NG = 4
NJ = 8
TM = 256
NB = S // TM
FC = 256
NFC = F // FC
EPS = 1e-5

bf16 = jnp.bfloat16
f32 = jnp.float32

_NT = (((1,), (1,)), ((), ()))


def _dot(a, b):
    return jnp.dot(a, b, preferred_element_type=f32)


def _dot_nt(a, b):
    return lax.dot_general(a, b, _NT, preferred_element_type=f32)


def _layernorm_mod(x, scale1p, shift):
    m = jnp.mean(x, axis=-1, keepdims=True)
    xc = x - m
    v = jnp.mean(xc * xc, axis=-1, keepdims=True)
    return xc * lax.rsqrt(v + EPS) * scale1p + shift


def _fold(x):
    return pltpu.roll(x, 4, 0)


def _feature_map_j(pT):
    n = pT.shape[-1]
    t = pT.reshape(8, 8, n)
    mx = jnp.max(t, axis=0)
    mx = jnp.maximum(mx, _fold(mx))
    mn = jnp.min(t, axis=0)
    mn = jnp.minimum(mn, _fold(mn))
    ep = jnp.exp(t - mx[None])
    en = jnp.exp(mn[None] - t)
    sp = jnp.sum(ep, axis=0)
    sp = sp + _fold(sp)
    sn = jnp.sum(en, axis=0)
    sn = sn + _fold(sn)
    return jnp.concatenate([(ep * (1.0 / sp)[None]).reshape(64, n), (en * (1.0 / sn)[None]).reshape(64, n)], axis=0)


def _mo(v, m):
    return v if isinstance(v, int) else pl.multiple_of(v, m)


def _kernel(x_hbm, wqkv_hbm, wphi_hbm, wo_hbm, wg_hbm, wu_hbm, wd_hbm, c_hbm, wmod_hbm,
            out_hbm,
            x_v, h_v, out_v, wqkv_v, wphi_v, wo_v, wg_v, wu_v, wd_v, c_v, wmod_v,
            wqT_v, wkT_v, wvT_v, kv_acc, z_acc, kvT_v, zb_v, mod_v, x1_v, h2_v,
            sem_x, sem_o, sem_w):
    cp_phi = pltpu.make_async_copy(wphi_hbm, wphi_v, sem_w.at[0])
    cp_wk = pltpu.make_async_copy(wqkv_hbm.at[:, pl.ds(D, D)], wqkv_v.at[:, pl.ds(D, D)], sem_w.at[1])
    cp_c = pltpu.make_async_copy(c_hbm, c_v, sem_w.at[2])
    cp_m0 = pltpu.make_async_copy(wmod_hbm.at[:, pl.ds(0, 2 * D)], wmod_v.at[:, pl.ds(0, 2 * D)], sem_w.at[3])
    cp_wv = pltpu.make_async_copy(wqkv_hbm.at[:, pl.ds(2 * D, D)], wqkv_v.at[:, pl.ds(2 * D, D)], sem_w.at[4])
    cp_wq = pltpu.make_async_copy(wqkv_hbm.at[:, pl.ds(0, D)], wqkv_v.at[:, pl.ds(0, D)], sem_w.at[5])
    cp_m1 = pltpu.make_async_copy(wmod_hbm.at[:, pl.ds(2 * D, 4 * D)], wmod_v.at[:, pl.ds(2 * D, 4 * D)], sem_w.at[6])
    cp_wo = pltpu.make_async_copy(wo_hbm, wo_v, sem_w.at[7])
    cp_wg = pltpu.make_async_copy(wg_hbm, wg_v, sem_w.at[8])
    cp_wu = pltpu.make_async_copy(wu_hbm, wu_v, sem_w.at[9])
    cp_wd = pltpu.make_async_copy(wd_hbm, wd_v, sem_w.at[10])

    def x_copy(i):
        return pltpu.make_async_copy(x_hbm.at[pl.ds(i * TM, TM)], x_v.at[pl.ds(i * TM, TM)], sem_x.at[i])

    def o_copy(i):
        return pltpu.make_async_copy(out_v.at[pl.ds(i * TM, TM)], out_hbm.at[pl.ds(i * TM, TM)], sem_o.at[i])

    cp_phi.start()
    cp_wk.start()
    x_copy(0).start()
    cp_c.start()
    cp_m0.start()
    cp_wv.start()
    for i in range(1, NB):
        x_copy(i).start()
    cp_wq.start()
    cp_m1.start()
    cp_wo.start()
    cp_wg.start()
    cp_wu.start()
    cp_wd.start()

    cp_phi.wait()
    B = wphi_v[...].reshape(DH * DH, H)
    r1 = lax.broadcasted_iota(jnp.int32, (D, H), 0)
    c1 = lax.broadcasted_iota(jnp.int32, (D, H), 1)
    E1 = jnp.where((r1 // 64) * 4 + (r1 % 4) == c1, 1.0, 0.0).astype(bf16)
    M1 = _dot_nt(E1, B)
    r2 = lax.broadcasted_iota(jnp.int32, (D, DH * DH), 0)
    c2 = lax.broadcasted_iota(jnp.int32, (D, DH * DH), 1)
    M1 = jnp.where(((r2 % 64) // 4) == (c2 % DH), M1, 0.0).astype(bf16)
    r3 = lax.broadcasted_iota(jnp.int32, (DH * DH, 128), 0)
    c3 = lax.broadcasted_iota(jnp.int32, (DH * DH, 128), 1)
    E2 = jnp.where((r3 // DH) == (c3 % DH), 1.0, 0.0).astype(bf16)
    PT = _dot(M1, E2)
    r4 = lax.broadcasted_iota(jnp.int32, (D, 128), 0)
    c4 = lax.broadcasted_iota(jnp.int32, (D, 128), 1)
    PT = jnp.where(((r4 % 128) // 64) * 4 + (r4 % 4) == (c4 // DH), PT, 0.0).astype(bf16)
    pts = [PT[g * 128:(g + 1) * 128] for g in range(NG)]

    cp_wk.wait()
    for g in range(NG):
        wkT_v[g * 128:(g + 1) * 128, :] = _dot_nt(
            pts[g], wqkv_v[:, D + g * 128:D + (g + 1) * 128]).astype(bf16)

    kv_acc[...] = jnp.zeros_like(kv_acc)
    z_acc[...] = jnp.zeros_like(z_acc)

    HT = TM // 2

    x_copy(0).wait()
    x0 = x_v[pl.ds(0, TM), :].astype(f32)
    m0_ = jnp.mean(x0, axis=-1, keepdims=True)
    xc0 = x0 - m0_
    v0_ = jnp.mean(xc0 * xc0, axis=-1, keepdims=True)
    xn0 = xc0 * lax.rsqrt(v0_ + EPS)

    cp_c.wait()
    cp_m0.wait()
    cf = c_v[...].astype(f32)
    sc = (cf * jax.nn.sigmoid(cf)).astype(bf16).astype(f32)
    s_col = jnp.broadcast_to(sc, (128, D)).T

    def matvec(t0, t1):
        for t in range(t0, t1):
            w = wmod_v[:, t * 128:(t + 1) * 128].astype(f32)
            mod_v[0:1, t * 128:(t + 1) * 128] = jnp.sum(w * s_col, axis=0, keepdims=True)

    matvec(0, 8)
    h_v[pl.ds(0, TM), :] = (xn0 * (1.0 + mod_v[0:1, D:2 * D]) + mod_v[0:1, 0:D]).astype(bf16)

    def ln1_part(i, p):
        r0 = _mo(i * TM + p * HT, HT)
        x = x_v[pl.ds(r0, HT), :].astype(f32)
        sa = mod_v[0:1, 0:D]
        ca = mod_v[0:1, D:2 * D]
        h_v[pl.ds(r0, HT), :] = _layernorm_mod(x, 1.0 + ca, sa).astype(bf16)

    def kv_block(i, nxt, first=False, extra=None):
        r0 = _mo(i * TM, TM)
        h = h_v[pl.ds(r0, TM), :]
        kT = _dot_nt(wkT_v[...], h)
        if first:
            cp_wv.wait()
            x_copy(1).wait()
            wvT_v[...] = wqkv_v[:, 2 * D:3 * D].astype(f32).T.astype(bf16)
        if nxt:
            ln1_part(i + 1, 0)
        vT = _dot_nt(wvT_v[...], h).astype(bf16)
        if nxt:
            ln1_part(i + 1, 1)
        if extra is not None:
            extra()
        for j in range(NJ):
            ph = _feature_map_j(kT[j * 64:(j + 1) * 64])
            zs = ph[:, 0:128]
            for jj in range(1, TM // 128):
                zs = zs + ph[:, jj * 128:(jj + 1) * 128]
            z_acc[j] += zs
            kv_acc[j] += _dot_nt(vT[j * 64:(j + 1) * 64], ph.astype(bf16))

    kv_block(0, True, first=True)

    def phase1(i, carry):
        x_copy(i + 1).wait()
        kv_block(i, True)
        return carry

    lax.fori_loop(1, NB - 1, phase1, 0)

    cp_wq.wait()
    cp_m1.wait()
    cp_wo.wait()

    def extra():
        for g in range(NG):
            wqT_v[g * 128:(g + 1) * 128, :] = _dot_nt(
                pts[g], wqkv_v[:, g * 128:(g + 1) * 128]).astype(bf16)
        matvec(8, 24)

    kv_block(NB - 1, False, extra=extra)

    rk = lax.broadcasted_iota(jnp.int32, (64, 128), 0)
    ck = lax.broadcasted_iota(jnp.int32, (64, 128), 1)
    kv_mask = (rk // DH) == (ck % 4)
    for j in range(NJ):
        kvT_v[j] = jnp.where(kv_mask, kv_acc[j], 0.0).astype(bf16)
        z = jnp.sum(z_acc[j], axis=-1, keepdims=True)
        zb_v[j] = jnp.broadcast_to(z, (128, TM))

    def attn_stages(i):
        r0 = _mo(i * TM, TM)
        h = h_v[pl.ds(r0, TM), :]
        qT = _dot_nt(wqT_v[...], h)
        yield
        oTs = []
        for j in range(NJ):
            ph = _feature_map_j(qT[j * 64:(j + 1) * 64])
            den = jnp.sum((ph * zb_v[j]).reshape(16, 8, TM), axis=0)
            den = den + _fold(den)
            rden = 1.0 / (den + 1e-6)
            num = _dot(kvT_v[j], ph.astype(bf16))
            num = num.reshape(4, DH, TM) * rden[0:4, None, :]
            oTs.append(num.reshape(64, TM))
            if j % 4 == 3:
                yield
        oT = jnp.concatenate(oTs, axis=0)
        o = oT.T.astype(bf16)
        yield
        attn = _dot(o, wo_v[...])
        yield
        ga = mod_v[0:1, 2 * D:3 * D]
        sb = mod_v[0:1, 3 * D:4 * D]
        cb = mod_v[0:1, 4 * D:5 * D]
        for p in range(2):
            rp = _mo(i * TM + p * HT, HT)
            x = x_v[pl.ds(rp, HT), :].astype(f32)
            x1 = x + ga * attn[p * HT:(p + 1) * HT]
            x1_v[pl.ds(rp, HT), :] = x1
            h2_v[pl.ds(rp, HT), :] = _layernorm_mod(x1, 1.0 + cb, sb).astype(bf16)
            yield

    NQ = 4
    QR = TM // NQ

    def oq_copy(q):
        r = (NB - 1) * TM + q * QR
        return pltpu.make_async_copy(out_v.at[pl.ds(r, QR)], out_hbm.at[pl.ds(r, QR)], sem_o.at[NB - 1 + q])

    def ffn_stages(i, last=False):
        r0 = _mo(i * TM, TM)
        h2 = h2_v[pl.ds(r0, TM), :]
        gb = mod_v[0:1, 5 * D:6 * D]
        acc = None
        for j in range(NFC):
            gt = _dot(h2, wg_v[:, j * FC:(j + 1) * FC])
            up = _dot(h2, wu_v[:, j * FC:(j + 1) * FC])
            a = (jax.nn.gelu(gt, approximate=True) * up).astype(bf16)
            if last and j == NFC - 1:
                for q in range(NQ):
                    d = _dot(a[q * QR:(q + 1) * QR], wd_v[j * FC:(j + 1) * FC, :])
                    rq = i * TM + q * QR
                    out_v[pl.ds(rq, QR), :] = (x1_v[pl.ds(rq, QR), :] + gb * (acc[q * QR:(q + 1) * QR] + d)).astype(bf16)
                    oq_copy(q).start()
                return
            d = _dot(a, wd_v[j * FC:(j + 1) * FC, :])
            acc = d if acc is None else acc + d
            if j < NFC - 1:
                yield
        out_v[pl.ds(r0, TM), :] = (x1_v[pl.ds(r0, TM), :] + gb * acc).astype(bf16)
        o_copy(i).start()
        yield

    for _ in attn_stages(0):
        pass
    cp_wg.wait()
    cp_wu.wait()
    cp_wd.wait()

    def phase2(i, carry):
        fs = ffn_stages(i)
        as_ = attn_stages(i + 1)
        done_a = done_f = False
        while not (done_a and done_f):
            if not done_a:
                try:
                    next(as_)
                except StopIteration:
                    done_a = True
            if not done_f:
                try:
                    next(fs)
                except StopIteration:
                    done_f = True
        return carry

    lax.fori_loop(0, NB - 1, phase2, 0)
    for _ in ffn_stages(NB - 1, last=True):
        pass

    for i in range(NB - 1):
        o_copy(i).wait()
    for q in range(NQ):
        oq_copy(q).wait()


@jax.jit
def pallas_adaLN_cond__linear_kernel_hedgehog__geglu_ffn__prompt_kernel(
    A_x, A_wqkv, A_w_phi, A_wo, B_x, B_w_gate, B_w_up, B_w_down, c, w_mod,
):
    x2 = A_x.reshape(S, D)
    wphiT = jnp.transpose(A_w_phi, (1, 2, 0))
    any_spec = pl.BlockSpec(memory_space=pl.ANY)
    out = pl.pallas_call(
        _kernel,
        out_shape=jax.ShapeDtypeStruct((S, D), bf16),
        in_specs=[any_spec] * 9,
        out_specs=any_spec,
        scratch_shapes=[
            pltpu.VMEM((S, D), bf16),
            pltpu.VMEM((S, D), bf16),
            pltpu.VMEM((S, D), bf16),
            pltpu.VMEM((D, 3 * D), bf16),
            pltpu.VMEM((DH, DH, H), bf16),
            pltpu.VMEM((D, D), bf16),
            pltpu.VMEM((D, F), bf16),
            pltpu.VMEM((D, F), bf16),
            pltpu.VMEM((F, D), bf16),
            pltpu.VMEM((1, D), bf16),
            pltpu.VMEM((D, 6 * D), bf16),
            pltpu.VMEM((D, D), bf16),
            pltpu.VMEM((D, D), bf16),
            pltpu.VMEM((D, D), bf16),
            pltpu.VMEM((NJ, 64, 128), f32),
            pltpu.VMEM((NJ, 128, 128), f32),
            pltpu.VMEM((NJ, 64, 128), bf16),
            pltpu.VMEM((NJ, 128, TM), f32),
            pltpu.VMEM((8, 6 * D), f32),
            pltpu.VMEM((S, D), f32),
            pltpu.VMEM((S, D), bf16),
            pltpu.SemaphoreType.DMA((NB,)),
            pltpu.SemaphoreType.DMA((NB + 3,)),
            pltpu.SemaphoreType.DMA((11,)),
        ],
        compiler_params=pltpu.CompilerParams(vmem_limit_bytes=100 * 1024 * 1024),
    )(x2, A_wqkv, wphiT, A_wo, B_w_gate, B_w_up, B_w_down, c, w_mod)
    return out.reshape(1, S, D)
```
